```python
import os as _os
_os.environ.setdefault("JAX_PLATFORMS", "cpu")
import jax
import jax.numpy as jnp

def _softmax(x, axis=-1):
    return jax.nn.softmax(x, axis=axis)
def _gelu(x):
    return jax.nn.gelu(x, approximate=True)
def _silu(x):
    return jax.nn.silu(x)
def _sigmoid(x):
    return jax.nn.sigmoid(x)
def _layernorm(x, axis=-1, eps=1e-5):
    m = jnp.mean(x, axis=axis, keepdims=True)
    v = jnp.var(x, axis=axis, keepdims=True)
    return (x - m) / jnp.sqrt(v + eps)
def _scatter_add(tgt, idx, src, axis=0):
    return tgt.at[idx].add(src)
def _segment_sum(src, seg, n):
    return jax.ops.segment_sum(src, seg, n)
class _Rng:
    def __init__(self, key):
        self._k = key
    def _next(self):
        self._k, sub = jax.random.split(self._k)
        return sub
    def normal(self, shape):
        return jax.random.normal(self._next(), shape, dtype=jnp.bfloat16)
    def randint(self, lo, hi, shape):
        return jax.random.randint(self._next(), shape, lo, hi, dtype=jnp.int32)
    def uniform(self, shape, lo=0.0, hi=1.0):
        return jax.random.uniform(self._next(), shape, jnp.bfloat16, lo, hi)
    def permutation(self, n):
        return jax.random.permutation(self._next(), n)


kernel_name = 'concat_heads__gqa_block_cached__mha_block_cached__near_ridge'

def setup_inputs():
    _rng = _Rng(jax.random.key(int.from_bytes(__import__("os").urandom(4), "little")))
    _w = (lambda a: (lambda t: t.astype(jnp.bfloat16) if jnp.issubdtype(t.dtype, jnp.floating) else t)(jnp.asarray(a)))
    def _A_setup():
        B, Sq, D = 16, 32, 1024
        Hq, Hkv, Sk, Dh = 32, 4, 32, 128
        assert Hq % Hkv == 0, (Hq, Hkv)
        return {
            "x": _w((lambda *s: _rng.normal(s) * 0.8)(B, Sq, D)),
            "k_cache": _w((lambda *s: _rng.normal(s) * 0.8)(B, Hkv, Sk, Dh)),
            "v_cache": _w((lambda *s: _rng.normal(s) * 0.05)(B, Hkv, Sk, Dh)),
            "wq": _w((lambda *s: _rng.normal(s) * 0.8)(D, Hq * Dh) * (D ** -0.5)),
            "wo": _w((lambda *s: _rng.normal(s) * 0.05)(Hq * Dh, D) * ((Hq * Dh) ** -0.5)),
        }
    _A_in = _A_setup()

    def _B_setup():
        B, Sq, D = 16, 32, 1024
        H, Sk, Dh = 32, 32, 128
        return {
            "x": _w((lambda *s: _rng.normal(s) * 0.8)(B, Sq, D)),
            "k_cache": _w((lambda *s: _rng.normal(s) * 0.8)(B, H, Sk, Dh)),
            "v_cache": _w((lambda *s: _rng.normal(s) * 0.05)(B, H, Sk, Dh)),
            "wq": _w((lambda *s: _rng.normal(s) * 0.8)(D, H * Dh) * (D ** -0.5)),
            "wo": _w((lambda *s: _rng.normal(s) * 0.05)(H * Dh, D) * ((H * Dh) ** -0.5)),
        }
    _B_in = _B_setup()

    return {
        "A_x": _A_in["x"],
        "A_k_cache": _A_in["k_cache"],
        "A_v_cache": _A_in["v_cache"],
        "A_wq": _A_in["wq"],
        "A_wo": _A_in["wo"],
        "B_x": _B_in["x"],
        "B_k_cache": _B_in["k_cache"],
        "B_v_cache": _B_in["v_cache"],
        "B_wq": _B_in["wq"],
        "B_wo": _B_in["wo"],
    }

def reference(A_x, A_k_cache, A_v_cache, A_wq, A_wo, B_x, B_k_cache, B_v_cache, B_wq, B_wo):
    def _A_ref(x, k_cache, v_cache, wq, wo):
        B, Sq, D = x.shape
        Hq, Dh = 32, 128
        Hkv = k_cache.shape[1]
        rep = Hq // Hkv
        q = (lambda x, *d: x.transpose(*d))((x @ wq).reshape(B, Sq, Hq, Dh), 0, 2, 1, 3)
        k = jnp.repeat(k_cache, rep, axis=1)
        v = jnp.repeat(v_cache, rep, axis=1)
        scores = jnp.einsum("bhqd,bhkd->bhqk", q, k) * (Dh ** -0.5)
        p = _softmax(scores, axis=-1)
        o = jnp.einsum("bhqk,bhkd->bhqd", p, v)
        return (lambda x, *d: x.transpose(*d))(o, 0, 2, 1, 3).reshape(B, Sq, Hq * Dh) @ wo

    def _B_ref(x, k_cache, v_cache, wq, wo):
        B, Sq, D = x.shape
        H, Dh = 32, 128
        q = (lambda x, *d: x.transpose(*d))((x @ wq).reshape(B, Sq, H, Dh), 0, 2, 1, 3)
        scores = jnp.einsum("bhqd,bhkd->bhqk", q, k_cache) * (Dh ** -0.5)
        p = _softmax(scores, axis=-1)
        o = jnp.einsum("bhqk,bhkd->bhqd", p, v_cache)
        return (lambda x, *d: x.transpose(*d))(o, 0, 2, 1, 3).reshape(B, Sq, H * Dh) @ wo

    a = _A_ref(A_x, A_k_cache, A_v_cache, A_wq, A_wo)
    b = _B_ref(B_x, B_k_cache, B_v_cache, B_wq, B_wo)
    return jnp.concatenate([a, b], axis=-1)
```

```python
import functools, math
import jax, jax.numpy as jnp
from jax import lax
import jax.experimental.pallas as pl
import jax.experimental.pallas.tpu as pltpu

B, SQ, D, H, DH, SK = 16, 32, 1024, 32, 128, 32
M = B*SQ
C_EXP = (DH ** -0.5) * math.log2(math.e)
F32, BF16 = jnp.float32, jnp.bfloat16
NT = (((1,), (1,)), ((), ()))

PROD = {
    1: ([(1,(0,0)), (1,(1,1))],  [(1,(0,0)), (1,(1,1))],  [(1,(0,0)), (1,(1,1))]),
    2: ([(1,(1,0)), (1,(1,1))],  [(1,(0,0))],             [(1,(1,0)), (-1,(1,1))]),
    3: ([(1,(0,0))],             [(1,(0,1)), (-1,(1,1))], [(1,(0,1)), (1,(1,1))]),
    4: ([(1,(1,1))],             [(1,(1,0)), (-1,(0,0))], [(1,(0,0)), (1,(1,0))]),
    5: ([(1,(0,0)), (1,(0,1))],  [(1,(1,1))],             [(-1,(0,0)), (1,(0,1))]),
    6: ([(1,(1,0)), (-1,(0,0))], [(1,(0,0)), (1,(0,1))],  [(1,(1,1))]),
    7: ([(1,(0,1)), (-1,(1,1))], [(1,(1,0)), (1,(1,1))],  [(1,(0,0))]),
}
NTERMS = {(0,0): 4, (0,1): 2, (1,0): 2, (1,1): 4}

def merge(main, *extras):
    ev = [((i + 0.5) / len(main), 0, i, t) for i, t in enumerate(main)]
    for k, (ts, lo, hi) in enumerate(extras):
        ev += [(lo + (hi - lo) * (i + 0.5) / len(ts), k + 1, i, t) for i, t in enumerate(ts)]
    ev.sort(key=lambda e: e[:3])
    for e in ev: e[3]()

def make(LQ=1, LO=2, PR=16, qk_rng=(0.08, 0.45), pv_rng=(0.52, 0.85), flags=None, order=(2,1,5,3,6,4,7), lazy=True, dbg=0):
    STR = [PROD[i] for i in order]
    def expand(get, side, lv):
        if lv == 0:
            yield get(0, 0); return
        h = 1 << (lv - 1)
        for prod in STR:
            @functools.cache
            def sub(i, j, prod=prod):
                t = prod[side]
                v = get(t[0][1][0]*h + i, t[0][1][1]*h + j)
                for s, b in t[1:]:
                    w = get(b[0]*h + i, b[1]*h + j)
                    v = v + w if s > 0 else v - w
                return v
            yield from expand(sub, side, lv - 1)
    def raw_block(r, side, lv):
        i = j = 0
        for l in range(lv):
            t = STR[(r // 7**(lv-1-l)) % 7][side]
            if len(t) > 1: return None
            i, j = 2*i + t[0][1][0], 2*j + t[0][1][1]
        return i, j
    def operands(load, side, lv):
        g = functools.cache(lambda i, j: load(i, j).astype(F32))
        for r, v in enumerate(expand(g, side, lv)):
            raw = raw_block(r, side, lv)
            yield v.astype(BF16) if raw is None else load(*raw).astype(BF16)

    def total(terms):
        terms = sorted(terms[:-1], key=lambda t: -t[0]) + terms[-1:]
        s0, v = terms[0]
        for s, w in terms[1:]:
            v = (v + w if s > 0 else v - w) if s0 > 0 else w - v
            assert s0 > 0 or s > 0
            s0 = 1
        return v
    class Combine:
        def __init__(self, lv, emit):
            self.lv, self.emit, self.n, self.part, self.cnt = lv, emit, 0, {}, {}
        def push(self, m):
            if self.lv == 0:
                self.emit(0, 0, m); return
            per = 7 ** (self.lv - 1)
            if self.n % per == 0:
                self.inner = Combine(self.lv - 1, functools.partial(self._acc, STR[self.n // per][2]))
            self.n += 1
            self.inner.push(m)
        def _acc(self, terms, i, j, v):
            h = 1 << (self.lv - 1)
            for s, b in terms:
                key = (b[0]*h + i, b[1]*h + j)
                p = self.part.setdefault(key, [])
                p.append((s, v))
                self.cnt[key] = self.cnt.get(key, 0) + 1
                if self.cnt[key] == NTERMS[b]: self.emit(*key, total(self.part.pop(key)))
                elif not lazy and len(p) > 1: self.part[key] = [(1, total(p))]

    NQ, RQ, NO, RO = 1 << LQ, 7 ** LQ, 1 << LO, 7 ** LO
    KQ = 8 // NQ
    def kern(xa, ka, va, wqa, woa, xb, kb, vb, wqb, wob, out,
             xs, w01, wqs, wos, kas, vas, kbs, vbs, xop, qx, qy, oop, acc, outs, sin, sout):
        lane_blk = lax.broadcasted_iota(jnp.int32, (SK, 128), 1) >> 5
        cp = pltpu.make_async_copy
        def xa_cp(s): return cp(xa.at[:, pl.ds(s*256, 256)], xs.at[0, :, pl.ds(s*256, 256)], sin.at[0, s])
        def w01_cp(s): return cp(wqa.at[pl.ds(s*256, 256), pl.ds(0, 1024)], w01.at[pl.ds(s*256, 256)], sin.at[0, 4 + s])
        def xb_cp(): return cp(xb, xs.at[1], sin.at[0, 8])
        def wq_cp(g, br=0):
            src = (wqa, wqb)[g // 8].at[:, pl.ds(g % 8 * 512, 512)] if isinstance(g, int) else wqa.at[:, pl.ds(0, 512)]
            return cp(src, wqs.at[g], sin.at[1, g])
        def wo_cp(u):
            src = (woa, wob)[u // 2].at[pl.ds(u % 2 * 2048, 2048)] if isinstance(u, int) else woa.at[pl.ds(0, 2048)]
            return cp(src, wos.at[u], sin.at[2, u])
        def kva_cp(w, g): return cp((ka, va)[w].at[:, g], (kas, vas)[w].at[g], sin.at[2, 4 + 4*w + g])
        def kvb_cp(w, u): return cp((kb, vb)[w].at[:, pl.ds(u*16, 16)], (kbs, vbs)[w].at[u], sin.at[2, 12 + 2*w + u])
        def out_cp(br, i, j):
            return cp(outs.at[br, i, j], out.at[pl.ds(i*256, 256), pl.ds(br*D + j*128, 128)], sout.at[br, i, j])
        def wait(*cs):
            if not dbg:
                for c in cs: c.wait()

        pend = []
        def flush():
            while pend: pend.pop(0)()

        def x_prep(br, ks):
            rm = M // NQ
            def task(k, p):
                for r, v in enumerate(operands(lambda i, j: xs[br, pl.ds(i*rm + p, PR), pl.ds((k*NQ + j)*128, 128)], 0, LQ)):
                    xop[br, r, k, pl.ds(p, PR), :] = v
            return [functools.partial(task, k, p) for k in ks for p in range(0, rm, PR)]

        def q_mm(br, g, dst, hook=None):
            rm = M // NQ
            tasks = []
            for s in range(4 // NQ):
                def emit(i, j, v, s=s): dst[0][dst[1], s*NQ + j, pl.ds(i*rm, rm), :] = v.astype(BF16)
                cmb = Combine(LQ, emit)
                def load(i, j, s=s):
                    return jnp.concatenate([wqs[g, pl.ds((k*NQ + i)*128, 128), pl.ds((s*NQ + j)*128, 128)] for k in range(KQ)], axis=0)
                ops = operands(load, 1, LQ)
                def task(r, cmb=cmb, ops=ops, s=s):
                    w = next(ops)
                    if hook and s == 4 // NQ - 1 and r == RQ - 1: hook()
                    flush()
                    lhs = jnp.concatenate([xop[br, r, k] for k in range(KQ)], axis=1)
                    pend.append(functools.partial(cmb.push, jnp.dot(lhs, w, preferred_element_type=F32)))
                tasks += [functools.partial(task, r) for r in range(RQ)]
            return tasks

        def attn(br, it, c, src):
            ps = {}
            def qk(b):
                q4 = jnp.concatenate([src[0][src[1], j, b*SQ:(b+1)*SQ, :] for j in range(4)], axis=0)
                if br == 0:
                    st = lax.dot_general(kas[2*it + c//2, b], q4, NT, preferred_element_type=F32)
                else:
                    k4 = jnp.concatenate([kbs[it, b, 4*c + j] for j in range(4)], axis=0)
                    full = lax.dot_general(k4, q4, NT, preferred_element_type=F32)
                    st = full[96:128]
                    for j in (2, 1, 0):
                        st = jnp.where(lane_blk == j, full[j*32:(j+1)*32], st)
                m = jnp.max(st, axis=0, keepdims=True)
                e = jnp.exp2((st - m) * C_EXP)
                return e * (1.0 / jnp.sum(e, axis=0, keepdims=True))
            def qk_unit(u):
                ps[u] = jnp.concatenate([qk(4*i + u) for i in range(4)], axis=0).T
            def pv_unit(u):
                p = ps.pop(u)
                o = []
                for j in range(4):
                    ph = p[j*32:(j+1)*32]
                    l = jnp.concatenate([jnp.where(lane_blk == i, ph, 0.0) for i in range(4)], axis=0).astype(BF16)
                    v4 = jnp.concatenate([vas[2*it + c//2, 4*i + u] if br == 0 else vbs[it, 4*i + u, 4*c + j] for i in range(4)], axis=0)
                    o.append(jnp.dot(l, v4, preferred_element_type=F32))
                def fin():
                    w = 4 // NO
                    for ii in range(w):
                        for jj in range(w):
                            for r, v in enumerate(operands(lambda i, j: o[j*w + jj][(i*w + ii)*SQ:(i*w + ii + 1)*SQ], 0, LO)):
                                oop[r, c*w + jj, pl.ds((ii*4 + u)*SQ, SQ), :] = v
                pend.append(fin)
            return [([functools.partial(qk_unit, u) for u in range(4)], *qk_rng), ([functools.partial(pv_unit, u) for u in range(4)], *pv_rng)]

        KO, NTL = 16 // NO, 8 // NO
        def o_mm(br, it, t, splits):
            rm, w = M // NO, 4 // NO
            done = {}
            def emit(i, j, v):
                n = j*NTL + t
                v = v + jnp.where(it > 0, acc[n, pl.ds(i*rm, rm), :], 0.0)
                acc[n, pl.ds(i*rm, rm), :] = v
                for q in range(max(1, rm // 256)):
                    hf, off = divmod(i*rm + q*256, 256)
                    outs[br, hf, n, pl.ds(off, min(rm, 256)), :] = v[q*256:(q+1)*256].astype(BF16)
                    done[hf, n] = done.get((hf, n), 0) + min(rm, 256)
                    if done[hf, n] == 256:
                        pl.when(it > 0)(out_cp(br, hf, n).start)
            cmb = Combine(LO, emit)
            part = {}
            res = []
            for ks in splits:
                def load(i, j, ks=ks):
                    return jnp.concatenate([wos[2*br + it, pl.ds((k//w*4 + i*w + k%w)*128, 128), pl.ds((j*NTL + t)*128, 128)] for k in ks], axis=0)
                ops = operands(load, 1, LO)
                def task(r, ks=ks, ops=ops):
                    wv = next(ops)
                    flush()
                    v = jnp.dot(jnp.concatenate([oop[r, k] for k in ks], axis=1), wv, preferred_element_type=F32)
                    if r in part: v = v + part.pop(r)
                    if ks is splits[-1]: pend.append(functools.partial(cmb.push, v))
                    else: part[r] = v
                res.append([functools.partial(task, r) for r in range(RO)])
            return res

        if dbg != 1:
            q = [c for s in range(4) for c in (xa_cp(s), w01_cp(s))]
            q += [wq_cp(2), kva_cp(0, 0), kva_cp(1, 0), wq_cp(3), kva_cp(0, 1), kva_cp(1, 1), wq_cp(4), wq_cp(5), wo_cp(0)]
            q += [xb_cp(), wq_cp(6), kva_cp(0, 2), kva_cp(1, 2), wq_cp(7), kva_cp(0, 3), kva_cp(1, 3), wq_cp(8), wq_cp(12), wo_cp(1)]
            for u in range(2):
                q += [wq_cp(9 + 4*u + i) for i in range(3)] + [kvb_cp(0, u), kvb_cp(1, u), wo_cp(2 + u)]
            for c in q[:4]: c.start()

        part = {}
        def emit0(i, j, v):
            for p in range(4):
                qx[j, p, pl.ds(i*256, 256), :] = v[:, p*128:(p+1)*128].astype(BF16)
        cmb = Combine(1, emit0)
        wait(xa_cp(0), w01_cp(0))
        if dbg != 1:
            for c in q[4:]: c.start()
        for s in range(4):
            aops = operands(lambda i, j: xs[0, pl.ds(i*256, 256), pl.ds((2*s + j)*128, 128)], 0, 1)
            bops = operands(lambda i, j: w01[pl.ds((2*s + i)*128, 128), pl.ds(j*512, 512)], 1, 1)
            for r in range(7):
                a, b = next(aops), next(bops)
                if LQ == 1: xop[0, r, s] = a
                if r == 6 and s < 3: wait(xa_cp(s + 1), w01_cp(s + 1))
                v = jnp.dot(a, b, preferred_element_type=F32)
                if s > 0: v = v + part[r]
                if s < 3: part[r] = v
                else: cmb.push(v)
            if LQ != 1:
                for t in x_prep(0, [k for k in range(KQ) if ((k + 1)*NQ - 1) // 2 == s]): t()

        def four(n): return [list(range(k, min(k + 4, n))) for k in range(0, n, 4)]
        def body_a(it, carry):
            wait(wq_cp(2 + 4*it), kva_cp(0, 2*it), kva_cp(1, 2*it))
            if not dbg: pl.when(it > 0)(xb_cp().wait)
            xt = x_prep(it, range(KQ))
            merge(q_mm(0, 2 + 4*it, (qy, 0), lambda: wait(wq_cp(3 + 4*it), kva_cp(0, 2*it + 1), kva_cp(1, 2*it + 1))),
                  *attn(0, it, 0, (qx, 0)), (xt[:len(xt)//2], 0.05, 0.9))
            merge(q_mm(0, 3 + 4*it, (qy, 1), lambda: wait(wq_cp(4 + 4*it), wq_cp(5 + 7*it))),
                  *attn(0, it, 1, (qx, 1)), (xt[len(xt)//2:], 0.05, 0.9))
            merge(q_mm(it, 4 + 4*it, (qx, 0)), *attn(0, it, 2, (qy, 0)))
            merge(q_mm(it, 5 + 7*it, (qx, 1), lambda: wait(wo_cp(it))), *attn(0, it, 3, (qy, 1)))
            for t in range(NTL):
                for ts in o_mm(0, it, t, four(KO)): merge(ts)
            flush()
            return carry
        lax.fori_loop(0, 2, body_a, 0)

        def body_b(it, carry):
            wait(*[wq_cp(9 + 4*it + i) for i in range(3)], kvb_cp(0, it), kvb_cp(1, it), wo_cp(2 + it))
            merge(q_mm(1, 9 + 4*it, (qy, 0)), *attn(1, it, 0, (qx, it)))
            merge(q_mm(1, 10 + 4*it, (qy, 1)), *attn(1, it, 1, (qy, 0)))
            merge(q_mm(1, 11 + 4*it, (qy, 2)), *attn(1, it, 2, (qy, 1)))
            if LO == 2:
                first, second = o_mm(1, it, 0, [[0, 1], [2, 3]])
                merge(first, *attn(1, it, 3, (qy, 2)))
                merge(second)
                t0 = 1
            else:
                a, b = o_mm(1, it, 0, four(KO)), o_mm(1, it, 1, four(KO))
                merge(a[0] + b[0], *attn(1, it, 3, (qy, 2)))
                for ts in a[1:] + b[1:]: merge(ts)
                t0 = 2
            for t in range(t0, NTL):
                for ts in o_mm(1, it, t, four(KO)): merge(ts)
            flush()
            return carry
        lax.fori_loop(0, 2, body_b, 0)
        for br in range(2):
            for i in range(2):
                for j in range(8): out_cp(br, i, j).wait()

    def fn(A_x, A_k, A_v, A_wq, A_wo, B_x, B_k, B_v, B_wq, B_wo):
        ANY = pl.BlockSpec(memory_space=pl.ANY)
        out = pl.pallas_call(
            kern, in_specs=[ANY]*10, out_specs=ANY,
            out_shape=jax.ShapeDtypeStruct((M, 2*D), BF16),
            scratch_shapes=[
                pltpu.VMEM((2, M, D), BF16), pltpu.VMEM((D, 1024), BF16),
                pltpu.VMEM((16, D, 512), BF16), pltpu.VMEM((4, 2048, D), BF16),
                pltpu.VMEM((4, B, SK, DH), BF16), pltpu.VMEM((4, B, SK, DH), BF16),
                pltpu.VMEM((2, B, 16, SK, DH), BF16), pltpu.VMEM((2, B, 16, SK, DH), BF16),
                pltpu.VMEM((2, RQ, KQ, M // NQ, 128), BF16),
                pltpu.VMEM((2, 4, M, DH), BF16), pltpu.VMEM((3, 4, M, DH), BF16),
                pltpu.VMEM((RO, 16 // NO, M // NO, 128), BF16),
                pltpu.VMEM((8, M, 128), F32),
                pltpu.VMEM((2, 2, 8, 256, 128), BF16),
                pltpu.SemaphoreType.DMA((3, 16)), pltpu.SemaphoreType.DMA((2, 2, 8)),
            ],
            compiler_params=pltpu.CompilerParams(vmem_limit_bytes=120<<20, disable_semaphore_checks=True, disable_bounds_checks=True, **({"flags": flags} if flags else {})),
        )(A_x.reshape(M, D), A_k, A_v, A_wq, A_wo, B_x.reshape(M, D), B_k, B_v, B_wq, B_wo)
        return out.reshape(B, SQ, 2*D)
    return fn


@jax.jit
def pallas_concat_heads__gqa_block_cached__mha_block_cached__near_ridge_kernel(
    A_x, A_k_cache, A_v_cache, A_wq, A_wo, B_x, B_k_cache, B_v_cache, B_wq, B_wo):
    return make(1, 2)(A_x, A_k_cache, A_v_cache, A_wq, A_wo, B_x, B_k_cache, B_v_cache, B_wq, B_wo)
```

```python
import functools
import math

import jax
import jax.numpy as jnp
from jax import lax
import jax.experimental.pallas as pl
import jax.experimental.pallas.tpu as pltpu

B, SQ, D, DH, SK = 16, 32, 1024, 128, 32
M = B * SQ
F32, BF16 = jnp.float32, jnp.bfloat16
SCALE_LOG2E = DH ** -0.5 * math.log2(math.e)

LHS, RHS, RES = 0, 1, 2
STRASSEN = {
    1: ([(1, 0, 0), (1, 1, 1)], [(1, 0, 0), (1, 1, 1)], [(1, 0, 0), (1, 1, 1)]),
    2: ([(1, 1, 0), (1, 1, 1)], [(1, 0, 0)], [(1, 1, 0), (-1, 1, 1)]),
    3: ([(1, 0, 0)], [(1, 0, 1), (-1, 1, 1)], [(1, 0, 1), (1, 1, 1)]),
    4: ([(1, 1, 1)], [(1, 1, 0), (-1, 0, 0)], [(1, 0, 0), (1, 1, 0)]),
    5: ([(1, 0, 0), (1, 0, 1)], [(1, 1, 1)], [(-1, 0, 0), (1, 0, 1)]),
    6: ([(1, 1, 0), (-1, 0, 0)], [(1, 0, 0), (1, 0, 1)], [(1, 1, 1)]),
    7: ([(1, 0, 1), (-1, 1, 1)], [(1, 1, 0), (1, 1, 1)], [(1, 0, 0)]),
}
OUTER = (2, 4, 1, 3, 6, 5, 7)
INNER = (2, 1, 5, 3, 6, 4, 7)
SWAP = {p: int(p in (2, 5, 6, 7)) for p in STRASSEN}


def _per_chunk(slots):
    return [49 * c + s for c, row in enumerate(slots) for s in row]


QK_AT = (
    _per_chunk([(5, 6, 9, 11, 13, 15, 18, 18), (5, 5, 8, 9, 15, 15, 20, 22),
                (5, 7, 8, 9, 13, 15, 18, 18), (3, 7, 8, 9, 13, 15, 15, 17)]),
    _per_chunk([(6, 6, 14, 15, 15, 16, 20, 21), (11, 12, 13, 14, 15, 16, 17, 19),
                (5, 6, 7, 8, 13, 14, 15, 16), (6, 9, 11, 13, 14, 14, 15, 16)]),
)
PV_AT = (
    _per_chunk([(21, 24, 27, 30, 33, 36, 43, 43), (21, 24, 28, 29, 33, 36, 36, 43),
                (20, 24, 27, 30, 33, 36, 43, 43), (21, 24, 27, 30, 33, 36, 43, 43)]),
    _per_chunk([(21, 22, 28, 29, 35, 37, 42, 43), (23, 29, 29, 30, 35, 38, 41, 43),
                (21, 28, 30, 36, 37, 41, 43, 46), (21, 22, 26, 31, 36, 36, 38, 39)]),
)
XB_AT = [r for r, n in enumerate(
    "3001210214011100403010310400014011010314000031110"
    "0131121222011000401203210400203030010203102031101") for _ in range(int(n))]

OUT_PARTS = [(0, n, 0, M) for n in range(8)] + [(1, n, 0, M) for n in range(4)] + [
    (1, 4 + j, i * 256 + r, rows)
    for i in range(2) for j in range(4)
    for r, rows in ([(0, 128), (128, 128)] if (i, j // 2) == (0, 0) else [(0, 256)])]

X_ROW = 16 * 2048


def _signed_sum(terms):
    terms = sorted(terms[:-1], key=lambda t: -t[0]) + terms[-1:]
    assert terms[0][0] > 0
    v = terms[0][1]
    for sign, w in terms[1:]:
        v = v + w if sign > 0 else v - w
    return v


def _operands(block, side, outer=OUTER):
    for p in outer:
        @functools.cache
        def sub(i, j, p=p):
            j ^= SWAP[p] if side == RHS else 0
            return _signed_sum([(s, block(2 * a + i, 2 * b + j, p)) for s, a, b in STRASSEN[p][side]])

        for q in INNER:
            yield _signed_sum([(s, sub(i, j)) for s, i, j in STRASSEN[q][side]])


def _combiner(emit, outer=OUTER):
    def level(done):
        pending = {}

        def add(p, key, v):
            for sign, i, j in STRASSEN[p][RES]:
                terms = pending.setdefault((i, j, key), [])
                terms.append((sign, v))
                if len(terms) == (4 if i == j else 2):
                    done(i, j, key, _signed_sum(pending.pop((i, j, key))))
        return add

    top = level(lambda a, b, ij, v: emit(2 * a + ij[0], 2 * b + ij[1], v))
    low = level(lambda i, j, p, v: top(p, (i, j ^ SWAP[p]), v))
    return lambda r, v: low(INNER[r % 7], outer[r // 7], v)


def _interleave(main, *extras):
    events = [(i + 0.5, 0, i, task) for i, task in enumerate(main)]
    for k, (tasks, slots) in enumerate(extras):
        assert len(tasks) == len(slots)
        events += [(slot, k + 1, i, task) for i, (task, slot) in enumerate(zip(tasks, slots))]
    for event in sorted(events, key=lambda e: e[:3]):
        event[3]()


def _mm(a, b, contract_b=0):
    return lax.dot_general(a, b, (((1,), (contract_b,)), ((), ())), preferred_element_type=F32)


def _kernel(xa, ka, va, wqa, woa, xb, kb, vb, wqb, wob, out,
            xs, wqs, wos, kas, vas, kbs, vbs, q_early, q_late, o0, o1, o2, o3, acc, outs,
            sem_q, sem_out, sem):
    o_ops = (o0, o1, o2, o3)
    lane_group = lax.broadcasted_iota(jnp.int32, (SK, 128), 1) >> 5

    def copy(src, dst, s):
        return pltpu.make_async_copy(dst if src is None else src, dst, s)

    def xa_cp(k, h):
        at = (slice(None), pl.ds(16 * h, 16), pl.ds(512 * k, 512))
        return copy(xa.at[at], xs.at[(0, *at)], sem.at[4 * k + h])

    def wq0_cp(k, h):
        rows = pl.ds(256 * h, 256)
        return copy(wqa.at[k, rows, pl.ds(0, 512)], wqs.at[0, k, rows], sem.at[8 + 2 * k + h])

    def wq1_cp(h):
        rows = pl.ds(256 * h, 256)
        return copy(wqa.at[:, rows, pl.ds(512, 512)], wqs.at[1, :, rows], sem.at[12 + h])

    def xb_cp():
        return copy(xb, xs.at[1], sem.at[14])

    def wq_cp(c):
        src = (wqa, wqb)[c // 8].at[:, :, pl.ds(c % 8 * 512, 512)] if isinstance(c, int) else None
        return copy(src, wqs.at[c], sem_q.at[c])

    def wo_cp(u, h):
        src = None
        if isinstance(u, int):
            src = (woa, wob)[u // 2].at[pl.ds(u % 2 * 2048, 2048), pl.ds((h ^ (1 - u % 2)) * 256, 256)]
        return copy(src, wos.at[pl.ds((4 * u + h) * 2048, 2048)], sem.at[16 + 4 * u + h])

    def kva_cp(w, u):
        return copy((ka, va)[w].at[:, pl.ds(2 * u, 2)], (kas, vas)[w].at[u], sem_q.at[16 + 2 * w + u])

    def kvb_cp(w, u):
        return copy((kb, vb)[w].at[:, pl.ds(16 * u, 16)], (kbs, vbs)[w].at[u], sem.at[32 + 2 * w + u])

    def out_cp(part):
        br, n, r0, rows = part
        return copy(outs.at[br, n, pl.ds(r0, rows)], out.at[pl.ds(r0, rows), pl.ds(br * D + n * 128, 128)],
                    sem_out.at[OUT_PARTS.index(part)])

    def start(*copies):
        for c in copies:
            c.start()

    def wait(*copies):
        for c in copies:
            c.wait()

    def start_on_trip(it, first, second=None):
        pl.when(it == 0)(first.start)
        if second is not None:
            pl.when(it > 0)(second.start)


    def x_op(br, p, q, row, rows):
        return wos.at[pl.ds(pl.multiple_of(X_ROW + (br * 49 + (p - 1) * 7 + q) * 128 + row, rows), rows)]

    def x_block(br, i, j, unit):
        k, r = divmod(unit, 8)
        return jnp.concatenate(
            [xs[br, 2 * i + h, pl.ds(8 * r, 8), pl.ds((4 * k + j) * 128, 128)].astype(F32) for h in range(2)],
            axis=1)

    def x_prepare(br, unit, block, outer):
        ops = _operands(block, LHS, outer)
        for p in outer:
            for q in range(7):
                x_op(br, p, q, 8 * unit, 8)[...] = next(ops).astype(BF16)

    def q_proj(br, c, dst, slot, it, outer=OUTER):
        swap = slot % 2 * 2

        def emit(i, j, v):
            dst[slot, j ^ swap, pl.ds(128 * i, 128), :] = v.astype(BF16)

        def block(i, j, p):
            return jnp.concatenate(
                [wqs[c + (it >> p), k, pl.ds(128 * i, 128), pl.ds((j ^ swap) * 128, 128)].astype(F32)
                 for k in range(2)], axis=0)

        push, ops = _combiner(emit, outer), _operands(block, RHS, outer)

        def product(r):
            lhs = jnp.concatenate(
                [jnp.concatenate([x_op(br, outer[r // 7], r % 7, 64 * k, 64)[:, pl.ds(128 * h, 128)]
                                  for h in range(2)], axis=0) for k in range(2)], axis=1)
            push(r, _mm(lhs, next(ops)))

        return [functools.partial(product, r) for r in range(49)]

    def attention(br, it, q_srcs):
        probs = {}

        def softmax_t(c, b):
            ref, slot = q_srcs[c]
            q = jnp.concatenate([ref[slot, j, pl.ds(b * SQ, SQ), :] for j in range(4)], axis=0)
            if br == 0:
                s = _mm(kas[it, b, c // 2], q, 1)
            else:
                full = _mm(jnp.concatenate([kbs[it, b, 4 * c + j] for j in range(4)], axis=0), q, 1)
                s = full[96:]
                for j in (2, 1, 0):
                    s = jnp.where(lane_group == j, full[32 * j:32 * (j + 1)], s)
            e = jnp.exp2((s - jnp.max(s, axis=0, keepdims=True)) * SCALE_LOG2E)
            return e * (1.0 / jnp.sum(e, axis=0, keepdims=True))

        def scores(c, u, h):
            if h == 0:
                probs[c, u] = [softmax_t(c, 4 * i + u) for i in (2, 3)]
            else:
                probs[c, u] = jnp.concatenate([softmax_t(c, 4 * i + u) for i in (0, 1)] + probs[c, u], axis=0).T

        def values(c, u, h):
            o = []
            for j in range(4):
                p = probs[c, u][32 * j + 16 * h:32 * j + 16 * (h + 1)]
                p = jnp.concatenate([jnp.where(lane_group[:16] == i, p, 0.0) for i in range(4)], axis=0)
                v = [vas[it, 4 * i + u, c // 2] if br == 0 else vbs[it, 4 * i + u, 4 * c + j] for i in range(4)]
                o.append(_mm(p.astype(BF16), jnp.concatenate(v, axis=0)))
            for r, v in enumerate(_operands(lambda i, j, _: o[j][16 * i:16 * (i + 1)], LHS)):
                o_ops[c][r, pl.ds(32 * u + 16 * h, 16), :] = v.astype(BF16)

        units = [(c, u, h) for c in range(4) for u in range(4) for h in range(2)]
        return (([functools.partial(scores, *a) for a in units], QK_AT[br]),
                ([functools.partial(values, *a) for a in units], PV_AT[br]))

    def out_proj(br, it, t, split=0):
        written, partial = set(), {}

        def emit(i, j, v):
            n, rows = 4 * t + j, pl.ds(128 * i, 128)
            v = v + jnp.where(it > 0, acc[0, n ^ 2, rows, :], 0.0)
            outs[br, n, rows, :] = v.astype(BF16)
            acc[it, n, rows, :] = v
            written.add((n, 128 * i))
            for part in OUT_PARTS:
                needed = range(part[2], part[2] + part[3], 128)
                if br == 1 and part[:2] == (1, n) and 128 * i in needed and all((n, r) in written for r in needed):
                    pl.when(it > 0)(out_cp(part).start)

        push = _combiner(emit)

        def products(chunks, lo, hi):
            def block(i, j, p):
                slab = 4 * (2 * br + it + (it >> p)) + 2 * t + j // 2
                return jnp.concatenate(
                    [wos[pl.ds(pl.multiple_of(slab * 2048 + (4 * c + i) * 128, 128), 128),
                         pl.ds(j % 2 * 128, 128)].astype(F32) for c in chunks], axis=0)

            ops = _operands(block, RHS, OUTER[lo:hi])

            def product(r):
                v = _mm(jnp.concatenate([o_ops[c][r] for c in chunks], axis=1), next(ops))
                if r in partial:
                    v = v + partial.pop(r)
                if 3 in chunks:
                    push(r, v)
                else:
                    partial[r] = v

            return [functools.partial(product, r) for r in range(7 * lo, 7 * hi)]

        return products((0, 1), 0, split), products((2, 3), 0, split), products((0, 1, 2, 3), split, 7)

    def prologue(it):
        partial = {}

        def piece(k, h, lo, hi):
            cols = pl.ds(512 * k + 256 * lo, 256 * (hi - lo))
            lhs = jnp.concatenate([xs[0, i, pl.ds(16 * h, 16), cols] for i in range(8)], axis=0)
            v = _mm(lhs, wqs[0, k, pl.ds(256 * lo, 256 * (hi - lo)), :])
            partial[h] = v = v + partial[h] if h in partial else v
            for unit in range(8 * k + 2 * h + lo, 8 * k + 2 * h + hi):
                once = functools.cache(lambda i, j, unit=unit: x_block(0, i, j, unit))
                x_prepare(0, unit, lambda i, j, _: once(i, j), OUTER)
            if k == 1 and hi == 2:
                for j in range(4):
                    for i in range(8):
                        q_early[0, j, pl.ds(64 * i + 16 * h, 16), :] = (
                            v[16 * i:16 * (i + 1), 128 * j:128 * (j + 1)].astype(BF16))

        for k in range(2):
            wait(wq0_cp(k, 0), xa_cp(k, 0))
            piece(k, 0, 0, 1)
            wait(wq0_cp(k, 1))
            piece(k, 0, 1, 2)
            for h in range(1, 4):
                wait(xa_cp(k, h))
                piece(k, h, 0, 2)
        _interleave(
            q_proj(0, 1, q_early, 1, it, (2, 6, 4, 1, 3, 5, 7)),
            ([lambda: wait(wq1_cp(0)), lambda: wait(wq1_cp(1))], [0, 14]),
            ([lambda: start(wq_cp(2)), lambda: start(kva_cp(0, 0), kva_cp(1, 0), wq_cp(3)),
              lambda: start(wq_cp(4)), lambda: start(wq_cp(5)),
              lambda: start(wo_cp(0, 0), wo_cp(0, 1), xb_cp(), wo_cp(0, 2), wo_cp(0, 3))], [0, 20, 27, 34, 49]))

    def branch_a(it, carry):
        pl.when(it == 0)(functools.partial(prologue, it))
        wait(wq_cp(2 + 4 * it))
        copies = [
            lambda: wait(kva_cp(0, it)),
            lambda: wait(kva_cp(1, it)),
            lambda: (start_on_trip(it, wq_cp(6), wq_cp(9)), wait(wq_cp(3 + 4 * it))),
            lambda: (start_on_trip(it, wq_cp(7), wq_cp(10)), wait(wq_cp(4 + 4 * it), wq_cp(5 + 7 * it))),
            lambda: start_on_trip(it, kva_cp(0, 1)),
            lambda: start_on_trip(it, wq_cp(8), wq_cp(11)),
            lambda: start_on_trip(it, wq_cp(12)),
            lambda: start_on_trip(it, kva_cp(1, 1)),
            lambda: (wait(wo_cp(it, 0), wo_cp(it, 1)), pl.when(it == 0)(xb_cp().wait)),
        ]
        _interleave(
            q_proj(0, 2 + 4 * it, q_late, 0, it) + q_proj(0, 3 + 4 * it, q_late, 1, it)
            + q_proj(it, 4 + 4 * it, q_early, 0, it) + q_proj(it, 5 + 7 * it, q_early, 1, it),
            (copies, [5, 21, 48, 97, 103, 146, 167, 168, 195]),
            *attention(0, it, [(q_early, 0), (q_early, 1), (q_late, 0), (q_late, 1)]))

        def xb_prepare(unit, p):
            x_prepare(1, unit, lambda i, j, p: x_block(1 + (it >> p), i, j, unit), (p,))

        copies = [lambda h=h: start_on_trip(it, wo_cp(1, h), wo_cp(2, h)) for h in range(4)]
        copies.append(lambda: (start(kvb_cp(0, it), kvb_cp(1, it)), wait(wo_cp(it, 2), wo_cp(it, 3))))
        _interleave(
            out_proj(0, it, 0)[2] + out_proj(0, it, 1)[2],
            ([functools.partial(xb_prepare, unit, p) for unit in range(16) for p in OUTER], XB_AT),
            (copies, [6, 13, 20, 27, 48]))
        return carry

    def branch_b(it, carry):
        wait(*[wq_cp(9 + 4 * it + i) for i in range(3)], kvb_cp(0, it), kvb_cp(1, it))
        left, right = out_proj(1, it, 0, 4), out_proj(1, it, 1, 3)
        copies = [lambda c=c: start_on_trip(it, wq_cp(c)) for c in (13, 14, 15)]
        copies.append(lambda: wait(*[wo_cp(2 + it, h) for h in range(4)]))
        copies += [lambda h=h: start_on_trip(it, wo_cp(3, h)) for h in range(4)]
        slots = [6, 48, 97, 146, 195, 202, 209, 216]
        _interleave(
            [task for i in range(3) for task in q_proj(1, 9 + 4 * it + i, q_late, i, it)]
            + left[0] + right[0] + right[1] + left[1] + left[2] + right[2],
            *attention(1, it, [(q_early, it), (q_late, 0), (q_late, 1), (q_late, 2)]),
            ([lambda n=n: pl.when(it > 0)(out_cp(OUT_PARTS[n]).start) for n in range(8)], slots),
            (copies, slots))
        return carry

    for k in range(2):
        start(wq0_cp(k, 0), xa_cp(k, 0), wq0_cp(k, 1), xa_cp(k, 1), xa_cp(k, 2), xa_cp(k, 3))
    start(wq1_cp(0), wq1_cp(1))
    lax.fori_loop(0, 2, branch_a, 0)
    lax.fori_loop(0, 2, branch_b, 0)
    wait(*[out_cp(part) for part in OUT_PARTS])


@jax.jit
def pallas_concat_heads__gqa_block_cached__mha_block_cached__near_ridge_kernel(
    A_x: jax.Array,
    A_k_cache: jax.Array,
    A_v_cache: jax.Array,
    A_wq: jax.Array,
    A_wo: jax.Array,
    B_x: jax.Array,
    B_k_cache: jax.Array,
    B_v_cache: jax.Array,
    B_wq: jax.Array,
    B_wo: jax.Array,
):
    in_hbm = pl.BlockSpec(memory_space=pl.ANY)
    out = pl.pallas_call(
        _kernel,
        in_specs=[in_hbm] * 10,
        out_specs=in_hbm,
        out_shape=jax.ShapeDtypeStruct((M, 2 * D), BF16),
        scratch_shapes=[
            pltpu.VMEM((2, 8, 64, D), BF16),
            pltpu.VMEM((16, 2, 512, 512), BF16),
            pltpu.VMEM((X_ROW + 2 * 49 * 128, 256), BF16),
            pltpu.VMEM((2, B, 2, SK, DH), BF16),
            pltpu.VMEM((2, B, 2, SK, DH), BF16),
            pltpu.VMEM((2, B, 16, SK, DH), BF16),
            pltpu.VMEM((2, B, 16, SK, DH), BF16),
            pltpu.VMEM((2, 4, M, DH), BF16),
            pltpu.VMEM((3, 4, M, DH), BF16),
            *[pltpu.VMEM((49, 128, DH), BF16)] * 4,
            pltpu.VMEM((2, 8, M, 128), F32),
            pltpu.VMEM((2, 8, M, 128), BF16),
            pltpu.SemaphoreType.DMA((20,)),
            pltpu.SemaphoreType.DMA((len(OUT_PARTS),)),
            pltpu.SemaphoreType.DMA((36,)),
        ],
        compiler_params=pltpu.CompilerParams(
            vmem_limit_bytes=100 * 1024 * 1024,
            disable_semaphore_checks=True,
            flags={"XLA_TPU_RESCHEDULE_DMA_DONES": True},
        ),
    )(A_x.reshape(8, 64, D), A_k_cache, A_v_cache, A_wq.reshape(2, 512, -1), A_wo,
      B_x.reshape(8, 64, D), B_k_cache, B_v_cache, B_wq.reshape(2, 512, -1), B_wo)
    return out.reshape(B, SQ, 2 * D)
```
